```python
import os as _os
_os.environ.setdefault("JAX_PLATFORMS", "cpu")
import jax
import jax.numpy as jnp

def _softmax(x, axis=-1):
    return jax.nn.softmax(x, axis=axis)
def _gelu(x):
    return jax.nn.gelu(x, approximate=True)
def _silu(x):
    return jax.nn.silu(x)
def _sigmoid(x):
    return jax.nn.sigmoid(x)
def _layernorm(x, axis=-1, eps=1e-5):
    m = jnp.mean(x, axis=axis, keepdims=True)
    v = jnp.var(x, axis=axis, keepdims=True)
    return (x - m) / jnp.sqrt(v + eps)
def _scatter_add(tgt, idx, src, axis=0):
    return tgt.at[idx].add(src)
def _segment_sum(src, seg, n):
    return jax.ops.segment_sum(src, seg, n)
class _Rng:
    def __init__(self, key):
        self._k = key
    def _next(self):
        self._k, sub = jax.random.split(self._k)
        return sub
    def normal(self, shape):
        return jax.random.normal(self._next(), shape, dtype=jnp.bfloat16)
    def randint(self, lo, hi, shape):
        return jax.random.randint(self._next(), shape, lo, hi, dtype=jnp.int32)
    def uniform(self, shape, lo=0.0, hi=1.0):
        return jax.random.uniform(self._next(), shape, jnp.bfloat16, lo, hi)
    def permutation(self, n):
        return jax.random.permutation(self._next(), n)


kernel_name = 'gated_mix__mha_block__mha_block__prompt'

def setup_inputs():
    _rng = _Rng(jax.random.key(int.from_bytes(__import__("os").urandom(4), "little")))
    _w = (lambda a: (lambda t: t.astype(jnp.bfloat16) if jnp.issubdtype(t.dtype, jnp.floating) else t)(jnp.asarray(a)))
    def _A_setup():
        B, S, D, H = 1, 2048, 448, 16
        return {
            "x": _w((lambda *s: _rng.normal(s) * 0.05)(B, S, D)),
            "wqkv": _w((lambda *s: _rng.normal(s) * 0.4)(D, 3 * D)),
            "wo": _w((lambda *s: _rng.normal(s) * 0.05)(D, D)),
        }
    _A_in = _A_setup()

    def _B_setup():
        B, S, D, H = 1, 2048, 448, 16
        return {
            "x": _w((lambda *s: _rng.normal(s) * 0.05)(B, S, D)),
            "wqkv": _w((lambda *s: _rng.normal(s) * 0.4)(D, 3 * D)),
            "wo": _w((lambda *s: _rng.normal(s) * 0.05)(D, D)),
        }
    _B_in = _B_setup()

    return {
        "A_x": _A_in["x"],
        "A_wqkv": _A_in["wqkv"],
        "A_wo": _A_in["wo"],
        "B_x": _B_in["x"],
        "B_wqkv": _B_in["wqkv"],
        "B_wo": _B_in["wo"],
        "gate_w": _w((lambda *s: _rng.normal(s) * 0.05)(448) * 16.0),
    }

def reference(A_x, A_wqkv, A_wo, B_x, B_wqkv, B_wo, gate_w):
    def _A_ref(x, wqkv, wo):
        B, S, D = x.shape
        H = 16
        Dh = D // H
        qkv = (lambda x, *d: x.transpose(*d))((x @ wqkv).reshape(B, S, 3, H, Dh), 2, 0, 3, 1, 4)
        q, k, v = qkv[0], qkv[1], qkv[2]
        scores = jnp.einsum("bhqd,bhkd->bhqk", q, k) * (Dh ** -0.5)
        p = _softmax(scores, axis=-1)
        o = jnp.einsum("bhqk,bhkd->bhqd", p, v)
        return (lambda x, *d: x.transpose(*d))(o, 0, 2, 1, 3).reshape(B, S, D) @ wo

    def _B_ref(x, wqkv, wo):
        B, S, D = x.shape
        H = 16
        Dh = D // H
        qkv = (lambda x, *d: x.transpose(*d))((x @ wqkv).reshape(B, S, 3, H, Dh), 2, 0, 3, 1, 4)
        q, k, v = qkv[0], qkv[1], qkv[2]
        scores = jnp.einsum("bhqd,bhkd->bhqk", q, k) * (Dh ** -0.5)
        p = _softmax(scores, axis=-1)
        o = jnp.einsum("bhqk,bhkd->bhqd", p, v)
        return (lambda x, *d: x.transpose(*d))(o, 0, 2, 1, 3).reshape(B, S, D) @ wo

    x = A_x
    g = _sigmoid((x * gate_w).sum(-1, keepdims=True))
    a = _A_ref(x, A_wqkv, A_wo)
    b = _B_ref(x, B_wqkv, B_wo)
    return g * a + (1 - g) * b
```

```python
import functools
import math

import jax
import jax.numpy as jnp
from jax import lax
import jax.experimental.pallas as pl
import jax.experimental.pallas.tpu as pltpu

S = 2048
D = 448
H = 16
DH = 28
DP = 32
NG = 8
TQ = 256
CH = 256

_NT = (((1,), (1,)), ((), ()))


def _kernel(x_ref, wq_ref, wk_ref, wvt_ref, wot_ref, gw_ref, o_ref,
            q_sc, k_sc, vt_sc, g_sc, ot_sc):
    i = pl.program_id(0)
    qscale = (DH ** -0.5) * math.log2(math.e)

    @pl.when(i == 0)
    def _prologue():
        def body(c, carry):
            r0 = pl.multiple_of(c * CH, CH)
            xc = x_ref[pl.ds(r0, CH), :]
            kc = jnp.dot(xc, wk_ref[...], preferred_element_type=jnp.float32)
            qc = jnp.dot(xc, wq_ref[...], preferred_element_type=jnp.float32) * qscale
            for g in range(NG):
                k_sc[g, pl.ds(r0, CH), :] = kc[:, g * 128:(g + 1) * 128].astype(jnp.bfloat16)
                q_sc[g, pl.ds(r0, CH), :] = qc[:, g * 128:(g + 1) * 128].astype(jnp.bfloat16)
            vt = lax.dot_general(wvt_ref[...], xc, _NT,
                                 preferred_element_type=jnp.float32)
            rows = lax.broadcasted_iota(jnp.int32, vt.shape, 0)
            vt = jnp.where((rows & (DP - 1)) == DH, 1.0, vt)
            vt_sc[c] = vt.astype(jnp.bfloat16)
            gl = lax.dot_general(gw_ref[...], xc, _NT,
                                 preferred_element_type=jnp.float32)
            g_sc[c] = jax.nn.sigmoid(gl)
            return carry
        lax.fori_loop(0, S // CH, body, 0)

    q0 = pl.multiple_of(i * TQ, TQ)
    gate = jnp.concatenate([g_sc[i * (TQ // CH) + c][0:1, :] for c in range(TQ // CH)], axis=1)
    lane = lax.broadcasted_iota(jnp.int32, (TQ, 128), 1)

    def group(g, carry):
        kg = k_sc[g]
        qg = q_sc[g, pl.ds(q0, TQ), :]
        gsel = jnp.where(g < NG // 2, gate, 1.0 - gate)
        for j in range(4):
            qm = jnp.where((lane >= j * DP) & (lane < (j + 1) * DP), qg, jnp.zeros_like(qg))
            st = lax.dot_general(kg, qm, _NT, preferred_element_type=jnp.float32)
            m = jnp.max(st, axis=0, keepdims=True)
            p = jnp.exp2(st - m).astype(jnp.bfloat16)
            r0 = pl.multiple_of(g * 128 + j * DP, DP)
            ot = None
            for c in range(S // CH):
                part = jnp.dot(vt_sc[c, pl.ds(r0, DP), :], p[c * CH:(c + 1) * CH, :],
                               preferred_element_type=jnp.float32)
                ot = part if ot is None else ot + part
            l = ot[DH:DH + 1, :]
            ot_sc[pl.ds(r0, DP), :] = (ot * (gsel / l)).astype(jnp.bfloat16)
        return carry

    lax.fori_loop(0, NG, group, 0)

    outt = jnp.dot(wot_ref[...], ot_sc[...], preferred_element_type=jnp.float32)
    o_ref[...] = outt.T[:, :D].astype(o_ref.dtype)


def _pad_heads(w):
    w = w.reshape(D, H, DH)
    w = jnp.pad(w, ((0, 0), (0, 0), (0, DP - DH)))
    return w.reshape(D, H * DP)


@jax.jit
def pallas_gated_mix__mha_block__mha_block__prompt_kernel(
    A_x: jax.Array,
    A_wqkv: jax.Array,
    A_wo: jax.Array,
    B_x: jax.Array,
    B_wqkv: jax.Array,
    B_wo: jax.Array,
    gate_w: jax.Array,
):
    x = A_x.reshape(S, D)
    wq = jnp.concatenate([_pad_heads(A_wqkv[:, 0:D]), _pad_heads(B_wqkv[:, 0:D])], axis=1)
    wk = jnp.concatenate([_pad_heads(A_wqkv[:, D:2 * D]), _pad_heads(B_wqkv[:, D:2 * D])], axis=1)
    wvt = jnp.concatenate([_pad_heads(A_wqkv[:, 2 * D:]), _pad_heads(B_wqkv[:, 2 * D:])], axis=1).T
    wot = jnp.concatenate([_pad_heads(A_wo.T), _pad_heads(B_wo.T)], axis=1)
    wot = jnp.pad(wot, ((0, 512 - D), (0, 0)))
    gw = jnp.pad(gate_w.reshape(1, D), ((0, 7), (0, 0)))

    full = lambda shape: pl.BlockSpec(shape, lambda i: (0,) * len(shape))
    out = pl.pallas_call(
        _kernel,
        grid=(S // TQ,),
        in_specs=[full((S, D)), full((D, 1024)), full((D, 1024)), full((1024, D)),
                  full((512, 1024)), full((8, D))],
        out_specs=pl.BlockSpec((TQ, D), lambda i: (i, 0)),
        out_shape=jax.ShapeDtypeStruct((S, D), jnp.bfloat16),
        scratch_shapes=[
            pltpu.VMEM((NG, S, 128), jnp.bfloat16),
            pltpu.VMEM((NG, S, 128), jnp.bfloat16),
            pltpu.VMEM((S // CH, 1024, CH), jnp.bfloat16),
            pltpu.VMEM((S // CH, 8, CH), jnp.float32),
            pltpu.VMEM((1024, TQ), jnp.bfloat16),
        ],
        compiler_params=pltpu.CompilerParams(
            dimension_semantics=("arbitrary",),
            vmem_limit_bytes=100 * 1024 * 1024),
    )(x, wq, wk, wvt, wot, gw)
    return out.reshape(1, S, D)
```

```python
import math

import jax
import jax.numpy as jnp
from jax import lax
import jax.experimental.pallas as pl
import jax.experimental.pallas.tpu as pltpu

S = 2048
D = 448
H = 16
DH = 28
DP = 32
NG = 8
TQ = 512
NQ = S // TQ
CH = 512
NC = S // CH
KC = 128
NK = S // KC
LAG = 1
GU = 2

_NT = (((1,), (1,)), ((), ()))
_F32 = jnp.float32
_BF16 = jnp.bfloat16


def _sel_t(t, lo, width):
    r = lax.broadcasted_iota(jnp.int32, (128, width), 0)
    c = lax.broadcasted_iota(jnp.int32, (128, width), 1)
    src = 112 * t + DH * (r >> 5) + (r & 31) - lo
    hit = (c == src) & ((r & 31) < DH)
    return jnp.where(hit, 1.0, 0.0).astype(_BF16)


def _eye(n):
    r = lax.broadcasted_iota(jnp.int32, (n, n), 0)
    c = lax.broadcasted_iota(jnp.int32, (n, n), 1)
    return jnp.where(r == c, 1.0, 0.0).astype(_BF16)


def _band(t, n):
    lo = 128 * ((112 * t) // 128)
    hi = min(n, 128 * (-(-(112 * t + 112) // 128)))
    return lo, hi


def _kernel(xt_hbm, wa_hbm, wb_hbm, woa_hbm, wob_hbm, gw_ref, o_ref,
            xt_ref, wa_ref, wb_ref, wo_ref, sems,
            wq_sc, wk_sc, wv_sc, wot_sc,
            qt_sc, k_sc, vt_sc, g_sc, ot_sc, s0_sc, s1_sc, s2_sc, s3_sc, m_sc, z_sc):
    i = pl.program_id(0)
    qscale = (DH ** -0.5) * math.log2(math.e)
    s_bufs = (s0_sc, s1_sc, s2_sc, s3_sc)

    def masked_qt(qb, g, j):
        r0 = pl.multiple_of(g * 128 + j * DP, DP)
        parts = []
        if j > 0:
            parts.append(jnp.zeros((j * DP, TQ), _BF16))
        parts.append(qt_sc[qb, pl.ds(r0, DP), :])
        if j < 3:
            parts.append(jnp.zeros(((3 - j) * DP, TQ), _BF16))
        return jnp.concatenate(parts, axis=0)

    def stage_a_chunk(g, qm, c, s_buf, m):
        st = jnp.dot(k_sc[g, c * KC:(c + 1) * KC, :], qm,
                     preferred_element_type=_F32)
        s_buf[c * KC:(c + 1) * KC, :] = st
        mc = jnp.max(st.reshape(KC // 8, 8, TQ), axis=0)
        return mc if m is None else jnp.maximum(m, mc)

    def stage_b_chunk(r0, c, s_buf, m, ot):
        z = z_sc[0]
        p = jnp.exp2(s_buf[pl.ds(pl.multiple_of(c * KC + z, KC), KC), :] - m).astype(_BF16)
        c0, c1 = divmod(c * KC, CH)
        part = jnp.dot(vt_sc[c0, pl.ds(r0, DP), c1:c1 + KC], p, preferred_element_type=_F32)
        return part if ot is None else ot + part

    @pl.when(i == 0)
    def _prologue():
        z_sc[0] = 0
        copies = [pltpu.make_async_copy(src, dst, sems.at[n]) for n, (src, dst) in enumerate(
            ((wa_hbm, wa_ref), (wb_hbm, wb_ref), (xt_hbm, xt_ref),
             (woa_hbm, wo_ref.at[0:D]), (wob_hbm, wo_ref.at[D:2 * D])))]
        for cp in copies:
            cp.start()

        eye = _eye(128)
        for b, w_ref in enumerate((wa_ref, wb_ref)):
            copies[b].wait()
            for dst, base in ((wq_sc, 0), (wv_sc, 2 * D)):
                for t in range(4):
                    n = min(128, D - 128 * t)
                    wt = lax.dot_general(eye[:n, :n], w_ref[:, base + 128 * t:base + 128 * t + n],
                                         _NT, preferred_element_type=_F32)
                    dst[b, 128 * t:128 * t + n, :] = wt.astype(_BF16)
            for t in range(4, 8):
                lo, hi = _band(t, 3 * D)
                wt = lax.dot_general(_sel_t(t, lo, hi - lo), w_ref[:, lo:hi], _NT,
                                     preferred_element_type=_F32)
                r0 = b * 512 + (t - 4) * 128
                wk_sc[r0:r0 + 128, :] = wt.astype(_BF16)

        gw = jnp.broadcast_to(gw_ref[...].reshape(1, D), (8, D))
        prow = lax.broadcasted_iota(jnp.int32, (DP - DH, CH), 0)
        vpad = jnp.where(prow == 0, 1.0, 0.0)
        qpad = jnp.zeros((DP - DH, CH), _F32)
        copies[2].wait()

        def body(c, carry):
            r0 = pl.multiple_of(c * CH, CH)
            xtc = xt_ref[:, pl.ds(r0, CH)]
            qb = c // (TQ // CH)
            l0 = pl.multiple_of((c % (TQ // CH)) * CH, CH)
            for b in range(2):
                qt = jnp.dot(wq_sc[b], xtc, preferred_element_type=_F32) * qscale
                vt = jnp.dot(wv_sc[b], xtc, preferred_element_type=_F32)
                for h in range(H):
                    d0 = (b * H + h) * DP
                    qh = jnp.concatenate([qt[h * DH:(h + 1) * DH], qpad], axis=0)
                    vh = jnp.concatenate([vt[h * DH:(h + 1) * DH], vpad], axis=0)
                    qt_sc[qb, d0:d0 + DP, pl.ds(l0, CH)] = qh.astype(_BF16)
                    vt_sc[c, d0:d0 + DP, :] = vh.astype(_BF16)
            gl = jnp.dot(gw, xtc, preferred_element_type=_F32)
            g_sc[c] = jax.nn.sigmoid(gl)
            xp = jnp.concatenate([xtc.astype(_F32), jnp.zeros((512 - D, CH), _F32)], axis=0)
            xc = xp.T[:, :D].astype(_BF16)
            kc = lax.dot_general(xc, wk_sc[...], _NT, preferred_element_type=_F32)
            for g in range(NG):
                k_sc[g, pl.ds(r0, CH), :] = kc[:, g * 128:(g + 1) * 128].astype(_BF16)
            return carry
        lax.fori_loop(0, NC, body, 0)

        copies[3].wait()
        copies[4].wait()
        for t in range(4):
            n = min(128, D - 128 * t)
            wt = lax.dot_general(eye[:n, :n], wo_ref[:, 128 * t:128 * t + n], _NT,
                                 preferred_element_type=_F32)
            wot_sc[128 * t:128 * t + n, :] = wt.astype(_BF16)

        qm = masked_qt(0, 0, 0)
        m = None
        for c in range(NK):
            m = stage_a_chunk(0, qm, c, s0_sc, m)
        m_sc[...] = m

    gate = jnp.concatenate([g_sc[i * (TQ // CH) + c][0:1, :] for c in range(TQ // CH)], axis=1)

    def group(gg, carry):
        nh = 4 * GU
        m8s = [m_sc[...]] + [None] * nh
        state = {}

        def a_step(t):
            h, c = divmod(t, NK)
            u, j = divmod(h, 4)
            g = gg * GU + u
            if c == 0:
                if j < 3:
                    qn, gn, jn = i, g, j + 1
                elif u < GU - 1:
                    qn, gn, jn = i, g + 1, 0
                else:
                    last = g == NG - 1
                    qn = jnp.where(last, jnp.minimum(i + 1, NQ - 1), i)
                    gn, jn = jnp.where(last, 0, g + 1), 0
                state['a'] = (gn, masked_qt(qn, gn, jn))
            gn, qm = state['a']
            m8s[h + 1] = stage_a_chunk(gn, qm, c, s_bufs[(h + 1) % 4], m8s[h + 1])

        def b_step(t):
            h, c = divmod(t, NK)
            u, j = divmod(h, 4)
            g = gg * GU + u
            if c == 0:
                state['m'] = jnp.max(m8s[h], axis=0, keepdims=True)
                state['ot'] = None
            r0 = pl.multiple_of(g * 128 + j * DP, DP)
            ot = stage_b_chunk(r0, c, s_bufs[h % 4], state['m'], state['ot'])
            state['ot'] = ot
            if c == NK - 1:
                gsel = jnp.where(g < NG // 2, gate, 1.0 - gate)
                l = ot[DH:DH + 1, :]
                ot_sc[g, j * DH:(j + 1) * DH, :] = (ot * (gsel / l))[:DH]

        nt = nh * NK
        for t in range(nt + LAG):
            if t < nt:
                a_step(t)
            if t >= LAG:
                b_step(t - LAG)
        m_sc[...] = m8s[nh]
        return carry

    lax.fori_loop(0, NG // GU, group, 0)

    o_all = ot_sc[...].reshape(NG * 4 * DH, TQ).astype(_BF16)
    outt = jnp.dot(wot_sc[...], o_all, preferred_element_type=_F32)
    o_ref[...] = outt.astype(o_ref.dtype)


@jax.jit
def pallas_gated_mix__mha_block__mha_block__prompt_kernel(
    A_x: jax.Array,
    A_wqkv: jax.Array,
    A_wo: jax.Array,
    B_x: jax.Array,
    B_wqkv: jax.Array,
    B_wo: jax.Array,
    gate_w: jax.Array,
):
    del B_x
    xt = A_x.reshape(S, D).T

    full = lambda shape: pl.BlockSpec(shape, lambda i: (0,) * len(shape))
    out_t = pl.pallas_call(
        _kernel,
        grid=(NQ,),
        in_specs=[pl.BlockSpec(memory_space=pl.ANY)] * 5 + [full((D,))],
        out_specs=pl.BlockSpec((D, TQ), lambda i: (0, i)),
        out_shape=jax.ShapeDtypeStruct((D, S), _BF16),
        scratch_shapes=[
            pltpu.VMEM((D, S), _BF16),
            pltpu.VMEM((D, 3 * D), _BF16),
            pltpu.VMEM((D, 3 * D), _BF16),
            pltpu.VMEM((2 * D, D), _BF16),
            pltpu.SemaphoreType.DMA((5,)),
            pltpu.VMEM((2, D, D), _BF16),
            pltpu.VMEM((1024, D), _BF16),
            pltpu.VMEM((2, D, D), _BF16),
            pltpu.VMEM((D, 2 * D), _BF16),
            pltpu.VMEM((NQ, 1024, TQ), _BF16),
            pltpu.VMEM((NG, S, 128), _BF16),
            pltpu.VMEM((NC, 1024, CH), _BF16),
            pltpu.VMEM((NC, 8, CH), _F32),
            pltpu.VMEM((NG, 4 * DH, TQ), _F32),
            pltpu.VMEM((S, TQ), _F32),
            pltpu.VMEM((S, TQ), _F32),
            pltpu.VMEM((S, TQ), _F32),
            pltpu.VMEM((S, TQ), _F32),
            pltpu.VMEM((8, TQ), _F32),
            pltpu.SMEM((1,), jnp.int32),
        ],
        compiler_params=pltpu.CompilerParams(
            dimension_semantics=("arbitrary",),
            vmem_limit_bytes=100 * 1024 * 1024),
    )(xt, A_wqkv, B_wqkv, A_wo, B_wo, gate_w)
    return out_t.T.reshape(1, S, D)
```

```python
import math

import jax
import jax.numpy as jnp
from jax import lax
import jax.experimental.pallas as pl
import jax.experimental.pallas.tpu as pltpu

S = 2048
D = 448
H = 16
DH = 28
DP = 32
NG = 8
TQ = 512
NQ = S // TQ
CH = 512
NC = S // CH
KC = 128
NK = S // KC
LAG = 1
GU = 2

_NT = (((1,), (1,)), ((), ()))
_F32 = jnp.float32
_BF16 = jnp.bfloat16


def _eye(n):
    r = lax.broadcasted_iota(jnp.int32, (n, n), 0)
    c = lax.broadcasted_iota(jnp.int32, (n, n), 1)
    return jnp.where(r == c, 1.0, 0.0).astype(_BF16)


def _kernel(xt_hbm, wa_hbm, wb_hbm, woa_hbm, wob_hbm, gw_ref, o_ref,
            xt_ref, wa_ref, wb_ref, wo_ref, sems,
            wt_sc, wot_sc,
            qt_sc, k_sc, vt_sc, g_sc, ot_sc, s0_sc, s1_sc, s2_sc, s3_sc, m_sc, z_sc):
    i = pl.program_id(0)
    qscale = (DH ** -0.5) * math.log2(math.e)
    s_bufs = (s0_sc, s1_sc, s2_sc, s3_sc)

    def masked_qt(qb, g, j):
        r0 = pl.multiple_of(g * 128 + j * DP, DP)
        parts = []
        if j > 0:
            parts.append(jnp.zeros((j * DP, TQ), _BF16))
        parts.append(qt_sc[qb, pl.ds(r0, DP), :])
        if j < 3:
            parts.append(jnp.zeros(((3 - j) * DP, TQ), _BF16))
        return jnp.concatenate(parts, axis=0)

    def stage_a_chunk(g, qm, c, s_buf, m):
        st = jnp.dot(k_sc[g, c * KC:(c + 1) * KC, :], qm,
                     preferred_element_type=_F32)
        s_buf[c * KC:(c + 1) * KC, :] = st
        mc = jnp.max(st.reshape(KC // 8, 8, TQ), axis=0)
        return mc if m is None else jnp.maximum(m, mc)

    def stage_b_chunk(r0, c, s_buf, m, ot):
        z = z_sc[0]
        p = jnp.exp2(s_buf[pl.ds(pl.multiple_of(c * KC + z, KC), KC), :] - m).astype(_BF16)
        c0, c1 = divmod(c * KC, CH)
        part = jnp.dot(vt_sc[c0, pl.ds(r0, DP), c1:c1 + KC], p, preferred_element_type=_F32)
        return part if ot is None else ot + part

    @pl.when(i == 0)
    def _prologue():
        z_sc[0] = 0
        def x_copy(c):
            cols = pl.ds(pl.multiple_of(c * CH, CH), CH)
            return pltpu.make_async_copy(xt_hbm.at[:, cols], xt_ref.at[:, cols], sems.at[4 + c])

        copies = [pltpu.make_async_copy(src, dst, sems.at[n]) for n, (src, dst) in enumerate(
            ((wa_hbm.at[:, 0:512], wa_ref.at[:, 0:512]), (wb_hbm, wb_ref),
             (woa_hbm, wo_ref.at[0:D]), (wob_hbm, wo_ref.at[D:2 * D])))]
        wa_rest = [pltpu.make_async_copy(wa_hbm.at[:, lo:hi], wa_ref.at[:, lo:hi],
                                         sems.at[4 + NC + n])
                   for n, (lo, hi) in enumerate(((512, 1024), (1024, 3 * D)))]
        copies[0].start()
        for cp in wa_rest:
            cp.start()
        for c in range(NC):
            x_copy(c).start()
        for cp in copies[1:]:
            cp.start()

        eye = _eye(128)
        prow = lax.broadcasted_iota(jnp.int32, (DP - DH, CH), 0)
        vpad = jnp.where(prow == 0, 1.0, 0.0)
        qpad = jnp.zeros((DP - DH, CH), _F32)
        wt_sc[0, 3 * D:3 * D + 16, :] = jnp.broadcast_to(gw_ref[...].reshape(1, D), (16, D))

        for b, w_ref in enumerate((wa_ref, wb_ref)):
            copies[b].wait()
            for t in range(11):
                if b == 0 and t in (4, 8):
                    wa_rest[t // 4 - 1].wait()
                lo, hi = 128 * t, min(128 * (t + 1), 3 * D)
                wt = lax.dot_general(eye[:hi - lo, :hi - lo], w_ref[:, lo:hi],
                                     _NT, preferred_element_type=_F32)
                wt_sc[b, lo:hi, :] = wt.astype(_BF16)

            def body(c, carry, b=b):
                if b == 0:
                    x_copy(c).wait()
                r0 = pl.multiple_of(c * CH, CH)
                xtc = xt_ref[:, pl.ds(r0, CH)]
                qb = c // (TQ // CH)
                l0 = pl.multiple_of((c % (TQ // CH)) * CH, CH)
                kt = jnp.dot(wt_sc[b, D:2 * D, :], xtc, preferred_element_type=_F32)
                for g in range(4):
                    kg = jnp.concatenate(
                        [piece for h in range(4 * g, 4 * g + 4)
                         for piece in (kt[h * DH:(h + 1) * DH], qpad)], axis=0)
                    k_sc[b * 4 + g, pl.ds(r0, CH), :] = kg.T.astype(_BF16)
                qt = jnp.dot(wt_sc[b, 0:D, :], xtc, preferred_element_type=_F32) * qscale
                vt = jnp.dot(wt_sc[b, 2 * D:3 * D + (16 if b == 0 else 0), :], xtc,
                             preferred_element_type=_F32)
                if b == 0:
                    g_sc[c] = jax.nn.sigmoid(vt[D:D + 8])
                for h in range(H):
                    d0 = (b * H + h) * DP
                    qh = jnp.concatenate([qt[h * DH:(h + 1) * DH], qpad], axis=0)
                    vh = jnp.concatenate([vt[h * DH:(h + 1) * DH], vpad], axis=0)
                    qt_sc[qb, d0:d0 + DP, pl.ds(l0, CH)] = qh.astype(_BF16)
                    vt_sc[c, d0:d0 + DP, :] = vh.astype(_BF16)
                return carry
            lax.fori_loop(0, NC, body, 0)

        copies[2].wait()
        copies[3].wait()
        for t in range(4):
            n = min(128, D - 128 * t)
            wt = lax.dot_general(eye[:n, :n], wo_ref[:, 128 * t:128 * t + n], _NT,
                                 preferred_element_type=_F32)
            wot_sc[128 * t:128 * t + n, :] = wt.astype(_BF16)

        qm = masked_qt(0, 0, 0)
        m = None
        for c in range(NK):
            m = stage_a_chunk(0, qm, c, s0_sc, m)
        m_sc[...] = m

    gate = jnp.concatenate([g_sc[i * (TQ // CH) + c][0:1, :] for c in range(TQ // CH)], axis=1)

    def group(gg, carry):
        nh = 4 * GU
        m8s = [m_sc[...]] + [None] * nh
        state = {}

        def a_step(t):
            h, c = divmod(t, NK)
            u, j = divmod(h, 4)
            g = gg * GU + u
            if c == 0:
                if j < 3:
                    qn, gn, jn = i, g, j + 1
                elif u < GU - 1:
                    qn, gn, jn = i, g + 1, 0
                else:
                    last = g == NG - 1
                    qn = jnp.where(last, jnp.minimum(i + 1, NQ - 1), i)
                    gn, jn = jnp.where(last, 0, g + 1), 0
                state['a'] = (gn, masked_qt(qn, gn, jn))
            gn, qm = state['a']
            m8s[h + 1] = stage_a_chunk(gn, qm, c, s_bufs[(h + 1) % 4], m8s[h + 1])

        def b_step(t):
            h, c = divmod(t, NK)
            u, j = divmod(h, 4)
            g = gg * GU + u
            if c == 0:
                state['m'] = jnp.max(m8s[h], axis=0, keepdims=True)
                state['ot'] = None
            r0 = pl.multiple_of(g * 128 + j * DP, DP)
            ot = stage_b_chunk(r0, c, s_bufs[h % 4], state['m'], state['ot'])
            state['ot'] = ot
            if c == NK - 1:
                gsel = jnp.where(g < NG // 2, gate, 1.0 - gate)
                l = ot[DH:DH + 1, :]
                ot_sc[g, j * DH:(j + 1) * DH, :] = (ot * (gsel / l))[:DH]

        nt = nh * NK
        for t in range(nt + LAG):
            if t < nt:
                a_step(t)
            if t >= LAG:
                b_step(t - LAG)
        m_sc[...] = m8s[nh]
        return carry

    lax.fori_loop(0, NG // GU, group, 0)

    o_all = ot_sc[...].reshape(NG * 4 * DH, TQ).astype(_BF16)
    outt = jnp.dot(wot_sc[...], o_all, preferred_element_type=_F32)
    o_ref[...] = outt.astype(o_ref.dtype)


@jax.jit
def pallas_gated_mix__mha_block__mha_block__prompt_kernel(
    A_x: jax.Array,
    A_wqkv: jax.Array,
    A_wo: jax.Array,
    B_x: jax.Array,
    B_wqkv: jax.Array,
    B_wo: jax.Array,
    gate_w: jax.Array,
):
    del B_x
    xt = A_x.reshape(S, D).T

    full = lambda shape: pl.BlockSpec(shape, lambda i: (0,) * len(shape))
    out_t = pl.pallas_call(
        _kernel,
        grid=(NQ,),
        in_specs=[pl.BlockSpec(memory_space=pl.ANY)] * 5 + [full((D,))],
        out_specs=pl.BlockSpec((D, TQ), lambda i: (0, i)),
        out_shape=jax.ShapeDtypeStruct((D, S), _BF16),
        scratch_shapes=[
            pltpu.VMEM((D, S), _BF16),
            pltpu.VMEM((D, 3 * D), _BF16),
            pltpu.VMEM((D, 3 * D), _BF16),
            pltpu.VMEM((2 * D, D), _BF16),
            pltpu.SemaphoreType.DMA((6 + NC,)),
            pltpu.VMEM((2, 3 * D + 16, D), _BF16),
            pltpu.VMEM((D, 2 * D), _BF16),
            pltpu.VMEM((NQ, 1024, TQ), _BF16),
            pltpu.VMEM((NG, S, 128), _BF16),
            pltpu.VMEM((NC, 1024, CH), _BF16),
            pltpu.VMEM((NC, 8, CH), _F32),
            pltpu.VMEM((NG, 4 * DH, TQ), _F32),
            pltpu.VMEM((S, TQ), _F32),
            pltpu.VMEM((S, TQ), _F32),
            pltpu.VMEM((S, TQ), _F32),
            pltpu.VMEM((S, TQ), _F32),
            pltpu.VMEM((8, TQ), _F32),
            pltpu.SMEM((1,), jnp.int32),
        ],
        compiler_params=pltpu.CompilerParams(
            dimension_semantics=("arbitrary",),
            vmem_limit_bytes=100 * 1024 * 1024),
    )(xt, A_wqkv, B_wqkv, A_wo, B_wo, gate_w)
    return out_t.T.reshape(1, S, D)
```
